```python
import os as _os
_os.environ.setdefault("JAX_PLATFORMS", "cpu")
import jax
import jax.numpy as jnp

def _softmax(x, axis=-1):
    return jax.nn.softmax(x, axis=axis)
def _gelu(x):
    return jax.nn.gelu(x, approximate=True)
def _silu(x):
    return jax.nn.silu(x)
def _sigmoid(x):
    return jax.nn.sigmoid(x)
def _layernorm(x, axis=-1, eps=1e-5):
    m = jnp.mean(x, axis=axis, keepdims=True)
    v = jnp.var(x, axis=axis, keepdims=True)
    return (x - m) / jnp.sqrt(v + eps)
def _scatter_add(tgt, idx, src, axis=0):
    return tgt.at[idx].add(src)
def _segment_sum(src, seg, n):
    return jax.ops.segment_sum(src, seg, n)
class _Rng:
    def __init__(self, key):
        self._k = key
    def _next(self):
        self._k, sub = jax.random.split(self._k)
        return sub
    def normal(self, shape):
        return jax.random.normal(self._next(), shape, dtype=jnp.bfloat16)
    def randint(self, lo, hi, shape):
        return jax.random.randint(self._next(), shape, lo, hi, dtype=jnp.int32)
    def uniform(self, shape, lo=0.0, hi=1.0):
        return jax.random.uniform(self._next(), shape, jnp.bfloat16, lo, hi)
    def permutation(self, n):
        return jax.random.permutation(self._next(), n)


kernel_name = 'concat_heads__gqa_block_cached__sliding_block_cached__decode'

def setup_inputs():
    _rng = _Rng(jax.random.key(int.from_bytes(__import__("os").urandom(4), "little")))
    _w = (lambda a: (lambda t: t.astype(jnp.bfloat16) if jnp.issubdtype(t.dtype, jnp.floating) else t)(jnp.asarray(a)))
    def _A_setup():
        B, Sq, D = 2, 1, 448
        Hq, Hkv, Sk, Dh = 16, 8, 8192, 256
        assert Hq % Hkv == 0, (Hq, Hkv)
        return {
            "x": _w((lambda *s: _rng.normal(s) * 0.8)(B, Sq, D)),
            "k_cache": _w((lambda *s: _rng.normal(s) * 0.8)(B, Hkv, Sk, Dh)),
            "v_cache": _w((lambda *s: _rng.normal(s) * 0.05)(B, Hkv, Sk, Dh)),
            "wq": _w((lambda *s: _rng.normal(s) * 0.8)(D, Hq * Dh) * (D ** -0.5)),
            "wo": _w((lambda *s: _rng.normal(s) * 0.05)(Hq * Dh, D) * ((Hq * Dh) ** -0.5)),
        }
    _A_in = _A_setup()

    def _B_setup():
        B, Sq, D = 2, 1, 448
        Hq, Hkv, Sk, Dh = 16, 8, 8192, 256
        assert Hq % Hkv == 0, (Hq, Hkv)
        return {
            "x": _w((lambda *s: _rng.normal(s) * 0.8)(B, Sq, D)),
            "k_cache": _w((lambda *s: _rng.normal(s) * 0.8)(B, Hkv, Sk, Dh)),
            "v_cache": _w((lambda *s: _rng.normal(s) * 0.05)(B, Hkv, Sk, Dh)),
            "wq": _w((lambda *s: _rng.normal(s) * 0.8)(D, Hq * Dh) * (D ** -0.5)),
            "wo": _w((lambda *s: _rng.normal(s) * 0.05)(Hq * Dh, D) * ((Hq * Dh) ** -0.5)),
        }
    _B_in = _B_setup()

    return {
        "A_x": _A_in["x"],
        "A_k_cache": _A_in["k_cache"],
        "A_v_cache": _A_in["v_cache"],
        "A_wq": _A_in["wq"],
        "A_wo": _A_in["wo"],
        "B_x": _B_in["x"],
        "B_k_cache": _B_in["k_cache"],
        "B_v_cache": _B_in["v_cache"],
        "B_wq": _B_in["wq"],
        "B_wo": _B_in["wo"],
    }

def reference(A_x, A_k_cache, A_v_cache, A_wq, A_wo, B_x, B_k_cache, B_v_cache, B_wq, B_wo):
    def _A_ref(x, k_cache, v_cache, wq, wo):
        B, Sq, D = x.shape
        Hq, Dh = 16, 256
        Hkv = k_cache.shape[1]
        rep = Hq // Hkv
        q = (lambda x, *d: x.transpose(*d))((x @ wq).reshape(B, Sq, Hq, Dh), 0, 2, 1, 3)
        k = jnp.repeat(k_cache, rep, axis=1)
        v = jnp.repeat(v_cache, rep, axis=1)
        scores = jnp.einsum("bhqd,bhkd->bhqk", q, k) * (Dh ** -0.5)
        p = _softmax(scores, axis=-1)
        o = jnp.einsum("bhqk,bhkd->bhqd", p, v)
        return (lambda x, *d: x.transpose(*d))(o, 0, 2, 1, 3).reshape(B, Sq, Hq * Dh) @ wo

    def _B_ref(x, k_cache, v_cache, wq, wo):
        B, Sq, D = x.shape
        Hq, Dh = 16, 256
        Hkv, Sk = k_cache.shape[1], k_cache.shape[2]
        W = min(4096, max(256, Sk // 4))
        rep = Hq // Hkv
        q = (lambda x, *d: x.transpose(*d))((x @ wq).reshape(B, Sq, Hq, Dh), 0, 2, 1, 3)
        k = jnp.repeat(k_cache[:, :, Sk - W:, :], rep, axis=1)
        v = jnp.repeat(v_cache[:, :, Sk - W:, :], rep, axis=1)
        scores = jnp.einsum("bhqd,bhkd->bhqk", q, k) * (Dh ** -0.5)
        p = _softmax(scores, axis=-1)
        o = jnp.einsum("bhqk,bhkd->bhqd", p, v)
        return (lambda x, *d: x.transpose(*d))(o, 0, 2, 1, 3).reshape(B, Sq, Hq * Dh) @ wo

    a = _A_ref(A_x, A_k_cache, A_v_cache, A_wq, A_wo)
    b = _B_ref(B_x, B_k_cache, B_v_cache, B_wq, B_wo)
    return jnp.concatenate([a, b], axis=-1)
```

```python
import jax
import jax.numpy as jnp
from jax import lax
import jax.experimental.pallas as pl
import jax.experimental.pallas.tpu as pltpu

_HQ, _DH = 16, 256
_CHUNK = 128
_AHEAD = 3
_DMA_HEADS = 2
_DMA_ROWS = 32
_W_HEADS = 2
_W_ROWS = 32
_NT = (((1,), (1,)), ((), ()))


@jax.jit
def pallas_concat_heads__gqa_block_cached__sliding_block_cached__decode_kernel(
    A_x: jax.Array,
    A_k_cache: jax.Array,
    A_v_cache: jax.Array,
    A_wq: jax.Array,
    A_wo: jax.Array,
    B_x: jax.Array,
    B_k_cache: jax.Array,
    B_v_cache: jax.Array,
    B_wq: jax.Array,
    B_wo: jax.Array,
):
    f32, bf16 = jnp.float32, jnp.bfloat16
    nb, _, d = A_x.shape
    hkv, sk_a = A_k_cache.shape[1], A_k_cache.shape[2]
    sk_b = B_k_cache.shape[2]
    window = min(4096, max(256, sk_b // 4))
    rep = _HQ // hkv
    scale = _DH ** -0.5
    steps_a, steps_b = sk_a // _CHUNK, window // _CHUNK
    total_a = nb * steps_a
    total = total_a + nb * steps_b
    nbuf = _AHEAD + 1
    wcols = _W_HEADS * _DH
    nw = _HQ // _W_HEADS
    rows = nb * _HQ

    def kernel_function(xa, ka, va, wqa, woa, xb, kb, vb, wqb, wob, o_ref,
                        kv_buf, x_buf, wq_buf, wo_buf, q_buf, m_buf, l_buf, acc_buf,
                        kv_sem, wq_sem, wo_sem, x_sem):
        def start_kv(k_hbm, v_hbm, b, row0, slot):
            for s in range(_CHUNK // _DMA_ROWS):
                for hg in range(hkv // _DMA_HEADS):
                    heads = pl.ds(hg * _DMA_HEADS, _DMA_HEADS)
                    for p, src in enumerate((k_hbm, v_hbm)):
                        pltpu.make_async_copy(
                            src.at[b, heads, pl.ds(row0 + s * _DMA_ROWS, _DMA_ROWS)],
                            kv_buf.at[slot, p, heads, pl.ds(s * _DMA_ROWS, _DMA_ROWS)],
                            kv_sem.at[slot],
                        ).start(priority=p)

        def start_a(j):
            row0 = pl.multiple_of((j % steps_a) * _CHUNK, _CHUNK)
            start_kv(ka, va, j // steps_a, row0, j % nbuf)

        def start_b(j):
            jj = j - total_a
            row0 = pl.multiple_of(sk_b - window + (jj % steps_b) * _CHUNK, _CHUNK)
            start_kv(kb, vb, jj // steps_b, row0, j % nbuf)

        def start_w(srcs, dst, sem, u):
            cols = pl.ds(pl.multiple_of(u * wcols, wcols), wcols)
            for r in range(d // _W_ROWS):
                for p, src in enumerate(srcs):
                    pltpu.make_async_copy(
                        src.at[pl.ds(r * _W_ROWS, _W_ROWS), cols],
                        dst.at[u, p, pl.ds(r * _W_ROWS, _W_ROWS)],
                        sem.at[u],
                    ).start(priority=p)

        def wait_all(buf, sem):
            pltpu.make_async_copy(buf, buf, sem).wait()

        for p, src in enumerate((xa, xb)):
            pltpu.make_async_copy(src, x_buf.at[p], x_sem.at[0]).start(priority=p)
        lax.fori_loop(0, _AHEAD, lambda u, _: start_w((wqa, wqb), wq_buf, wq_sem, u), None)

        m_buf[...] = jnp.full(m_buf.shape, -jnp.inf, f32)
        l_buf[...] = jnp.zeros(l_buf.shape, f32)
        acc_buf[...] = jnp.zeros(acc_buf.shape, f32)
        wait_all(x_buf, x_sem.at[0])

        x_batch = lax.broadcasted_iota(jnp.int32, (rows, d), 0) // _HQ
        x_rows = []
        for br in range(2):
            x = x_buf[br].astype(f32)
            xr = jnp.broadcast_to(x[0:1, :], (rows, d))
            for b in range(1, nb):
                xr = jnp.where(x_batch == b, x[b:b + 1, :], xr)
            x_rows.append(xr.astype(bf16))

        def q_step(u, q):
            @pl.when(u + _AHEAD < nw)
            def _():
                start_w((wqa, wqb), wq_buf, wq_sem, u + _AHEAD)

            @pl.when(u + _AHEAD >= nw)
            def _():
                start_a(u + _AHEAD - nw)

            wait_all(wq_buf.at[u], wq_sem.at[u])
            head = lax.broadcasted_iota(jnp.int32, (rows, _DH), 0) % _HQ
            out = []
            for br in range(2):
                qb = q[br]
                for t in range(_W_HEADS):
                    qh = jnp.dot(x_rows[br], wq_buf[u, br, :, t * _DH:(t + 1) * _DH],
                                 preferred_element_type=f32)
                    qb = jnp.where(head == u * _W_HEADS + t, qh, qb)
                out.append(qb)
            return tuple(out)

        q = lax.fori_loop(0, nw, q_step, (jnp.zeros((rows, _DH), f32),) * 2)
        for br in range(2):
            for b in range(nb):
                q_buf[br * nb + b] = q[br][b * _HQ:(b + 1) * _HQ].astype(bf16)

        def attn_step(i, _):
            j = i + _AHEAD

            @pl.when(j < total_a)
            def _():
                start_a(j)

            @pl.when(jnp.logical_and(j >= total_a, j < total))
            def _():
                start_b(j)

            @pl.when(j >= total)
            def _():
                start_w((woa, wob), wo_buf, wo_sem, j - total)

            slot = i % nbuf
            g = jnp.where(i < total_a, i // steps_a, nb + (i - total_a) // steps_b)
            wait_all(kv_buf.at[slot], kv_sem.at[slot])

            qg = q_buf[g]
            kv_head = lax.broadcasted_iota(jnp.int32, (_HQ, _CHUNK), 0) // rep
            s = None
            for h in range(hkv):
                sh = lax.dot_general(qg, kv_buf[slot, 0, h], _NT, preferred_element_type=f32)
                s = sh if s is None else jnp.where(kv_head == h, sh, s)
            s = s * scale
            m_old = m_buf[g]
            m_new = jnp.maximum(m_old, jnp.max(s, axis=1, keepdims=True))
            alpha = jnp.exp(m_old - m_new)
            p = jnp.exp(s - m_new)
            m_buf[g] = m_new
            l_buf[g] = alpha * l_buf[g] + p
            pv = None
            for h in range(hkv):
                ph = jnp.where(kv_head == h, p, 0.0).astype(bf16)
                t = jnp.dot(ph, kv_buf[slot, 1, h], preferred_element_type=f32)
                pv = t if pv is None else pv + t
            acc_buf[g] = jnp.tile(alpha, (1, _DH // _CHUNK)) * acc_buf[g] + pv

        lax.fori_loop(0, total, attn_step, None)

        o = []
        for br in range(2):
            l = jnp.concatenate([l_buf[br * nb + b] for b in range(nb)], axis=0)
            acc = jnp.concatenate([acc_buf[br * nb + b] for b in range(nb)], axis=0)
            o.append((acc / jnp.sum(l, axis=1, keepdims=True)).astype(bf16))

        def o_step(u, r):
            @pl.when(u + _AHEAD < nw)
            def _():
                start_w((woa, wob), wo_buf, wo_sem, u + _AHEAD)

            wait_all(wo_buf.at[u], wo_sem.at[u])
            head = lax.broadcasted_iota(jnp.int32, (rows, d), 0) % _HQ
            out = []
            for br in range(2):
                rb = r[br]
                for t in range(_W_HEADS):
                    rh = lax.dot_general(o[br], wo_buf[u, br, :, t * _DH:(t + 1) * _DH], _NT,
                                         preferred_element_type=f32)
                    rb = jnp.where(head == u * _W_HEADS + t, rh, rb)
                out.append(rb)
            return tuple(out)

        r = lax.fori_loop(0, nw, o_step, (jnp.zeros((rows, d), f32),) * 2)
        outs = [
            jnp.concatenate(
                [jnp.sum(r[br][b * _HQ:(b + 1) * _HQ], axis=0, keepdims=True) for b in range(nb)],
                axis=0)
            for br in range(2)
        ]
        o_ref[...] = jnp.concatenate(outs, axis=1).astype(o_ref.dtype)

    out = pl.pallas_call(
        kernel_function,
        out_shape=jax.ShapeDtypeStruct((nb, 2 * d), bf16),
        in_specs=[pl.BlockSpec(memory_space=pltpu.HBM)] * 10,
        out_specs=pl.BlockSpec(memory_space=pltpu.VMEM),
        scratch_shapes=[
            pltpu.VMEM((nbuf, 2, hkv, _CHUNK, _DH), bf16),
            pltpu.VMEM((2, nb, d), bf16),
            pltpu.VMEM((nw, 2, d, wcols), bf16),
            pltpu.VMEM((nw, 2, d, wcols), bf16),
            pltpu.VMEM((2 * nb, _HQ, _DH), bf16),
            pltpu.VMEM((2 * nb, _HQ, _CHUNK), f32),
            pltpu.VMEM((2 * nb, _HQ, _CHUNK), f32),
            pltpu.VMEM((2 * nb, _HQ, _DH), f32),
            pltpu.SemaphoreType.DMA((nbuf,)),
            pltpu.SemaphoreType.DMA((nw,)),
            pltpu.SemaphoreType.DMA((nw,)),
            pltpu.SemaphoreType.DMA((1,)),
        ],
        compiler_params=pltpu.CompilerParams(
            vmem_limit_bytes=48 * 1024 * 1024,
            disable_bounds_checks=True,
        ),
    )(
        A_x.reshape(nb, d), A_k_cache, A_v_cache, A_wq, A_wo.T,
        B_x.reshape(nb, d), B_k_cache, B_v_cache, B_wq, B_wo.T,
    )
    return out.reshape(nb, 1, 2 * d)
```

```python
import jax
import jax.numpy as jnp
import numpy as np
from jax import lax
import jax.experimental.pallas as pl
import jax.experimental.pallas.tpu as pltpu

_HQ, _DH = 16, 256
_CHUNK = 128
_AHEAD = 5
_DMA_HEADS, _DMA_ROWS = 2, 32
_COPY_ELEMS = 16384
_STREAMS = 4
_LAG = 28
_WO_BLOCK, _WO_STEP = 1024, 512
_WO_TAIL = (512, 256, 128, 128)
_WO_ISSUED = (44, 52, 60, 80, 88, 106, 113)
_NT = (((1,), (1,)), ((), ()))


def _wo_schedule(d):
    n_lead = (_HQ * _DH - sum(_WO_TAIL)) // _WO_BLOCK
    widths = (_WO_BLOCK,) * n_lead + _WO_TAIL
    starts = tuple(sum(widths[:u]) for u in range(len(widths)))
    assert sum(widths) == _HQ * _DH
    needed = []
    for u, (c0, nc) in enumerate(zip(starts, widths)):
        nr = min(_COPY_ELEMS // nc, d // 4)
        assert d % nr == 0 and nr % 8 == 0
        count = d // nr
        streams = max(s for s in range(1, _STREAMS + 1) if count % s == 0)
        for i in range(count // streams):
            for j in range(streams):
                for br in range(2):
                    needed.append((u, br, (i + j * count // streams) * nr, nr, c0, nc))
    n_pairs = len(needed) // 2
    landing = sorted((t + p * _LAG, p, t) for t in range(n_pairs) for p in range(2))
    pairs = [[None, None] for _ in range(n_pairs)]
    for copy, (_, p, t) in zip(needed, landing):
        pairs[t][p] = copy
        if copy[0] < n_lead:
            assert t < _WO_ISSUED[1 + copy[0] * (_WO_BLOCK // _WO_STEP)]
    assert len(_WO_ISSUED) == 1 + n_lead * (_WO_BLOCK // _WO_STEP)
    assert _WO_ISSUED[-1] == n_pairs
    return n_lead, starts, widths, pairs


@jax.jit
def pallas_concat_heads__gqa_block_cached__sliding_block_cached__decode_kernel(
    A_x: jax.Array,
    A_k_cache: jax.Array,
    A_v_cache: jax.Array,
    A_wq: jax.Array,
    A_wo: jax.Array,
    B_x: jax.Array,
    B_k_cache: jax.Array,
    B_v_cache: jax.Array,
    B_wq: jax.Array,
    B_wo: jax.Array,
):
    f32, bf16 = jnp.float32, jnp.bfloat16
    nb, _, d = A_x.shape
    hkv, sk_a = A_k_cache.shape[1], A_k_cache.shape[2]
    sk_b = B_k_cache.shape[2]
    window = min(4096, max(256, sk_b // 4))
    rep = _HQ // hkv
    scale = _DH ** -0.5
    steps_a, steps_b = sk_a // _CHUNK, window // _CHUNK
    total_a = nb * steps_a
    total = total_a + nb * steps_b
    nbuf = _AHEAD + 1
    rows = nb * _HQ
    n_lead, wo_starts, wo_widths, wo_pairs = _wo_schedule(d)
    d_pad = pl.cdiv(d, 128) * 128
    wo_row0 = (0, 2 * d - d_pad)
    assert sk_a % _CHUNK == 0 and window % _CHUNK == 0 and sk_b % _CHUNK == 0
    assert window <= sk_b and total_a >= _AHEAD and wo_row0[1] % 128 == 0

    def kernel_function(xa, ka, va, wqa, woa, xb, kb, vb, wqb, wob, o_ref,
                        kv_buf, x_buf, wq_buf, wo_buf, q_buf, m_buf, l_buf, acc_buf,
                        kv_sem, wo_sem, x_sem, wq_sem):
        def start_kv(k_hbm, v_hbm, b, row0, slot):
            for s in range(_CHUNK // _DMA_ROWS):
                for hg in range(hkv // _DMA_HEADS):
                    heads = pl.ds(hg * _DMA_HEADS, _DMA_HEADS)
                    for p, src in enumerate((k_hbm, v_hbm)):
                        pltpu.make_async_copy(
                            src.at[b, heads, pl.ds(row0 + s * _DMA_ROWS, _DMA_ROWS)],
                            kv_buf.at[slot, p, heads, pl.ds(s * _DMA_ROWS, _DMA_ROWS)],
                            kv_sem.at[slot],
                        ).start(priority=p)

        def start_a(j):
            row0 = pl.multiple_of((j % steps_a) * _CHUNK, _CHUNK)
            start_kv(ka, va, j // steps_a, row0, j % nbuf)

        def start_b(j):
            jj = j - total_a
            row0 = pl.multiple_of(sk_b - window + (jj % steps_b) * _CHUNK, _CHUNK)
            start_kv(kb, vb, jj // steps_b, row0, j % nbuf)

        def start_wo(lo, hi):
            for pair in wo_pairs[lo:hi]:
                for p, (u, br, r0, nr, c0, nc) in enumerate(pair):
                    pltpu.make_async_copy(
                        (woa, wob)[br].at[pl.ds(r0, nr), pl.ds(c0, nc)],
                        wo_buf.at[pl.ds(br * d + r0, nr), pl.ds(c0, nc)],
                        wo_sem.at[u],
                    ).start(priority=p)

        wq_cols = _COPY_ELEMS // 8
        wq_seg = d // _STREAMS
        wq_groups = (wq_seg // 8) * (_HQ * _DH // wq_cols)

        def start_wq(*branch_and_group):
            for j in range(_STREAMS):
                for p, i in branch_and_group:
                    rs = pl.ds(pl.multiple_of((i % (wq_seg // 8)) * 8 + j * wq_seg, 8), 8)
                    cs = pl.ds(pl.multiple_of((i // (wq_seg // 8)) * wq_cols, wq_cols), wq_cols)
                    pltpu.make_async_copy(
                        (wqa, wqb)[p].at[rs, cs], wq_buf.at[p, rs, cs], wq_sem.at[0],
                    ).start(priority=p)

        def wait_all(buf, sem):
            pltpu.make_async_copy(buf, buf, sem).wait()

        for br, src in enumerate((xa, xb)):
            pltpu.make_async_copy(src, x_buf.at[br], x_sem.at[0]).start()
        lead = _LAG // _STREAMS
        lax.fori_loop(0, lead, lambda i, _: start_wq((1, i)), None)
        lax.fori_loop(lead, wq_groups, lambda i, _: start_wq((0, i - lead), (1, i)), None)
        lax.fori_loop(wq_groups - lead, wq_groups, lambda i, _: start_wq((0, i)), None)
        lax.fori_loop(0, _AHEAD - 2, lambda j, _: start_a(j), None)

        m_buf[...] = jnp.full(m_buf.shape, np.finfo(np.float32).min, f32)
        l_buf[...] = jnp.zeros(l_buf.shape, f32)
        acc_buf[...] = jnp.zeros(acc_buf.shape, f32)

        wait_all(x_buf, x_sem.at[0])
        wait_all(wq_buf, wq_sem.at[0])
        x_batch = lax.broadcasted_iota(jnp.int32, (rows, d), 0) // _HQ
        q_head = lax.broadcasted_iota(jnp.int32, (rows, _DH), 0) % _HQ
        for br in range(2):
            x = x_buf[br].astype(f32)
            x_rows = jnp.broadcast_to(x[0:1, :], (rows, d))
            for b in range(1, nb):
                x_rows = jnp.where(x_batch == b, x[b:b + 1, :], x_rows)

            def q_step(h, q, br=br, lhs=x_rows.astype(bf16)):
                w = wq_buf[br, :, pl.ds(pl.multiple_of(h * _DH, _DH), _DH)]
                return jnp.where(q_head == h, jnp.dot(lhs, w, preferred_element_type=f32), q)

            q = lax.fori_loop(0, _HQ, q_step, jnp.zeros((rows, _DH), f32), unroll=4)
            for b in range(nb):
                q_buf[br * nb + b] = q[b * _HQ:(b + 1) * _HQ].astype(bf16)
            start_a(jnp.int32(_AHEAD - 2 + br))

        def attn_step(i, _):
            j = i + _AHEAD

            @pl.when(j < total_a)
            def _():
                start_a(j)

            @pl.when(jnp.logical_and(j >= total_a, j < total))
            def _():
                start_b(j)

            @pl.when(j >= total)
            def _():
                for t in range(_AHEAD):
                    @pl.when(j == total + t)
                    def _():
                        start_wo(t * _WO_ISSUED[0] // _AHEAD, (t + 1) * _WO_ISSUED[0] // _AHEAD)

            slot = i % nbuf
            g = jnp.where(i < total_a, i // steps_a, nb + (i - total_a) // steps_b)
            wait_all(kv_buf.at[slot], kv_sem.at[slot])

            qg = q_buf[g]
            kv_head = lax.broadcasted_iota(jnp.int32, (_HQ, _CHUNK), 0) // rep
            s = None
            for h in range(hkv):
                sh = lax.dot_general(qg, kv_buf[slot, 0, h], _NT, preferred_element_type=f32)
                s = sh if s is None else jnp.where(kv_head == h, sh, s)
            s = s * scale
            m_old = m_buf[g]
            m_new = jnp.maximum(m_old, jnp.max(s, axis=1, keepdims=True))
            alpha = jnp.exp(m_old - m_new)
            p = jnp.exp(s - m_new)
            m_buf[g] = m_new
            l_buf[g] = alpha * l_buf[g] + p
            pv = None
            for h in range(hkv):
                ph = jnp.where(kv_head == h, p, 0.0).astype(bf16)
                t = jnp.dot(ph, kv_buf[slot, 1, h], preferred_element_type=f32)
                pv = t if pv is None else pv + t
            acc_buf[g] = jnp.tile(alpha, (1, _DH // _CHUNK)) * acc_buf[g] + pv

        lax.fori_loop(0, total, attn_step, None)

        for g in range(2 * nb):
            acc_buf[g] = acc_buf[g] / jnp.sum(l_buf[g], axis=1, keepdims=True)

        def o_cols(br, c, n):
            w = min(n, _DH)
            lanes = slice(0, _DH) if n >= _DH else slice(c % _DH, c % _DH + n)
            row = lax.broadcasted_iota(jnp.int32, (8, w), 0)
            parts = []
            for t in range(n // w):
                part = jnp.zeros((8, w), f32)
                for b in range(nb):
                    head = acc_buf[br * nb + b, pl.ds(c // _DH + t, 1), lanes]
                    part = jnp.where(row == b, head, part)
                parts.append(part.astype(bf16))
            return jnp.concatenate(parts, axis=1)

        def project(r, o, c, n):
            return tuple(
                r[br] + lax.dot_general(o[br], wo_buf[pl.ds(wo_row0[br], d_pad), pl.ds(c, n)],
                                        _NT, preferred_element_type=f32)
                for br in range(2))

        per_block = _WO_BLOCK // _WO_STEP

        def o_step(k, r):
            for t in range(n_lead * per_block):
                @pl.when(k == t)
                def _():
                    start_wo(_WO_ISSUED[t], _WO_ISSUED[t + 1])

            c = pl.multiple_of(k * _WO_STEP, _WO_STEP)
            o = [o_cols(br, c, _WO_STEP) for br in range(2)]

            @pl.when(k % per_block == 0)
            def _():
                u = k // per_block
                cols = pl.ds(pl.multiple_of(u * _WO_BLOCK, _WO_BLOCK), _WO_BLOCK)
                wait_all(wo_buf.at[:, cols], wo_sem.at[u])

            return project(r, o, c, _WO_STEP)

        r = lax.fori_loop(0, n_lead * per_block, o_step, (jnp.zeros((8, d_pad), f32),) * 2)
        for u in range(n_lead, len(wo_widths)):
            c, n = wo_starts[u], wo_widths[u]
            o = [o_cols(br, c, n) for br in range(2)]
            wait_all(wo_buf.at[:, pl.ds(c, n)], wo_sem.at[u])
            r = project(r, o, c, n)

        lo = wo_row0[1]
        lane = lax.broadcasted_iota(jnp.int32, (8, d_pad - lo), 1)
        mid = jnp.where(lane < d - lo, r[0][:, lo:], r[1][:, :d_pad - lo])
        res = jnp.concatenate([r[0][:, :lo], mid, r[1][:, d_pad - lo:]], axis=1)
        o_ref[...] = res[:nb].astype(o_ref.dtype)

    out = pl.pallas_call(
        kernel_function,
        out_shape=jax.ShapeDtypeStruct((nb, 2 * d), bf16),
        in_specs=[pl.BlockSpec(memory_space=pltpu.HBM)] * 10,
        out_specs=pl.BlockSpec(memory_space=pltpu.VMEM),
        scratch_shapes=[
            pltpu.VMEM((nbuf, 2, hkv, _CHUNK, _DH), bf16),
            pltpu.VMEM((2, nb, d), bf16),
            pltpu.VMEM((2, d, _HQ * _DH), bf16),
            pltpu.VMEM((2 * d, _HQ * _DH), bf16),
            pltpu.VMEM((2 * nb, _HQ, _DH), bf16),
            pltpu.VMEM((2 * nb, _HQ, _CHUNK), f32),
            pltpu.VMEM((2 * nb, _HQ, _CHUNK), f32),
            pltpu.VMEM((2 * nb, _HQ, _DH), f32),
            pltpu.SemaphoreType.DMA((nbuf,)),
            pltpu.SemaphoreType.DMA((len(wo_widths),)),
            pltpu.SemaphoreType.DMA((1,)),
            pltpu.SemaphoreType.DMA((1,)),
        ],
        compiler_params=pltpu.CompilerParams(
            vmem_limit_bytes=32 * 1024 * 1024,
            disable_semaphore_checks=True,
        ),
    )(
        A_x.reshape(nb, d), A_k_cache, A_v_cache, A_wq, A_wo.T,
        B_x.reshape(nb, d), B_k_cache, B_v_cache, B_wq, B_wo.T,
    )
    return out.reshape(nb, 1, 2 * d)
```

```python
import jax
import jax.numpy as jnp
import numpy as np
from jax import lax
import jax.experimental.pallas as pl
import jax.experimental.pallas.tpu as pltpu

_HQ, _DH = 16, 256
_CHUNK = 128
_AHEAD = 5
_DMA_HEADS, _DMA_ROWS = 2, 32
_COPY_ELEMS = 16384
_STREAMS = 4
_LAG = 28
_WO_BLOCK, _WO_STEP = 1024, 512
_WO_TAIL = (512, 256, 128, 128)
_WO_ISSUED = (44, 52, 60, 80, 88, 106, 113)
_NT = (((1,), (1,)), ((), ()))


def _wo_schedule(d):
    n_lead = (_HQ * _DH - sum(_WO_TAIL)) // _WO_BLOCK
    widths = (_WO_BLOCK,) * n_lead + _WO_TAIL
    starts = tuple(sum(widths[:u]) for u in range(len(widths)))
    assert sum(widths) == _HQ * _DH
    needed = []
    for u, (c0, nc) in enumerate(zip(starts, widths)):
        nr = min(_COPY_ELEMS // nc, d // 4)
        assert d % nr == 0 and nr % 8 == 0
        count = d // nr
        streams = max(s for s in range(1, _STREAMS + 1) if count % s == 0)
        for i in range(count // streams):
            for j in range(streams):
                for br in range(2):
                    needed.append((u, br, (i + j * count // streams) * nr, nr, c0, nc))
    n_pairs = len(needed) // 2
    landing = sorted((t + p * _LAG, p, t) for t in range(n_pairs) for p in range(2))
    pairs = [[None, None] for _ in range(n_pairs)]
    for copy, (_, p, t) in zip(needed, landing):
        pairs[t][p] = copy
        if copy[0] < n_lead:
            assert t < _WO_ISSUED[1 + copy[0] * (_WO_BLOCK // _WO_STEP)]
    assert len(_WO_ISSUED) == 1 + n_lead * (_WO_BLOCK // _WO_STEP)
    assert _WO_ISSUED[-1] == n_pairs
    return n_lead, starts, widths, pairs


@jax.jit
def pallas_concat_heads__gqa_block_cached__sliding_block_cached__decode_kernel(
    A_x: jax.Array,
    A_k_cache: jax.Array,
    A_v_cache: jax.Array,
    A_wq: jax.Array,
    A_wo: jax.Array,
    B_x: jax.Array,
    B_k_cache: jax.Array,
    B_v_cache: jax.Array,
    B_wq: jax.Array,
    B_wo: jax.Array,
):
    f32, bf16 = jnp.float32, jnp.bfloat16
    nb, _, d = A_x.shape
    hkv, sk_a = A_k_cache.shape[1], A_k_cache.shape[2]
    sk_b = B_k_cache.shape[2]
    window = min(4096, max(256, sk_b // 4))
    rep = _HQ // hkv
    scale = _DH ** -0.5
    steps_a, steps_b = sk_a // _CHUNK, window // _CHUNK
    total_a = nb * steps_a
    total = total_a + nb * steps_b
    nbuf = _AHEAD + 1
    rows = nb * _HQ
    n_lead, wo_starts, wo_widths, wo_pairs = _wo_schedule(d)
    d_pad = pl.cdiv(d, 128) * 128
    wo_row0 = (0, 2 * d - d_pad)
    assert sk_a % _CHUNK == 0 and window % _CHUNK == 0 and sk_b % _CHUNK == 0
    assert window <= sk_b and total_a >= _AHEAD and wo_row0[1] % 128 == 0

    def kernel_function(xa, ka, va, wqa, woa, xb, kb, vb, wqb, wob, o_ref,
                        kv_buf, x_buf, wq_buf, wo_buf, q_buf, m_buf, l_buf, acc_buf,
                        kv_sem, wo_sem, x_sem, wq_sem):
        def start_kv(k_hbm, v_hbm, b, row0, slot):
            for s in range(_CHUNK // _DMA_ROWS):
                for hg in range(hkv // _DMA_HEADS):
                    heads = pl.ds(hg * _DMA_HEADS, _DMA_HEADS)
                    for p, src in enumerate((k_hbm, v_hbm)):
                        pltpu.make_async_copy(
                            src.at[b, heads, pl.ds(row0 + s * _DMA_ROWS, _DMA_ROWS)],
                            kv_buf.at[slot, p, heads, pl.ds(s * _DMA_ROWS, _DMA_ROWS)],
                            kv_sem.at[slot],
                        ).start(priority=p)

        def start_a(j):
            row0 = (j % steps_a) * _CHUNK
            if not isinstance(j, int):
                row0 = pl.multiple_of(row0, _CHUNK)
            start_kv(ka, va, j // steps_a, row0, j % nbuf)

        def start_b(j):
            jj = j - total_a
            row0 = pl.multiple_of(sk_b - window + (jj % steps_b) * _CHUNK, _CHUNK)
            start_kv(kb, vb, jj // steps_b, row0, j % nbuf)

        def start_wo(lo, hi):
            for pair in wo_pairs[lo:hi]:
                for p, (u, br, r0, nr, c0, nc) in enumerate(pair):
                    pltpu.make_async_copy(
                        (woa, wob)[br].at[pl.ds(r0, nr), pl.ds(c0, nc)],
                        wo_buf.at[pl.ds(br * d + r0, nr), pl.ds(c0, nc)],
                        wo_sem.at[u],
                    ).start(priority=p)

        wq_cols = _COPY_ELEMS // 8
        wq_seg = d // _STREAMS
        wq_groups = (wq_seg // 8) * (_HQ * _DH // wq_cols)

        def start_wq(*branch_and_group):
            for j in range(_STREAMS):
                for p, i in branch_and_group:
                    rs = pl.ds(pl.multiple_of((i % (wq_seg // 8)) * 8 + j * wq_seg, 8), 8)
                    cs = pl.ds(pl.multiple_of((i // (wq_seg // 8)) * wq_cols, wq_cols), wq_cols)
                    pltpu.make_async_copy(
                        (wqa, wqb)[p].at[rs, cs], wq_buf.at[p, rs, cs], wq_sem.at[0],
                    ).start(priority=p)

        def wait_all(buf, sem):
            pltpu.make_async_copy(buf, buf, sem).wait()

        for br, src in enumerate((xa, xb)):
            pltpu.make_async_copy(src, x_buf.at[br], x_sem.at[0]).start()
        lead = _LAG // _STREAMS
        lax.fori_loop(0, lead, lambda i, _: start_wq((1, i)), None)
        lax.fori_loop(lead, wq_groups, lambda i, _: start_wq((0, i - lead), (1, i)), None)
        lax.fori_loop(wq_groups - lead, wq_groups, lambda i, _: start_wq((0, i)), None)
        lax.fori_loop(0, _AHEAD - 2, lambda j, _: start_a(j), None)

        m_buf[...] = jnp.full(m_buf.shape, np.finfo(np.float32).min, f32)
        l_buf[...] = jnp.zeros(l_buf.shape, f32)
        acc_buf[...] = jnp.zeros(acc_buf.shape, f32)

        wait_all(x_buf, x_sem.at[0])
        wait_all(wq_buf, wq_sem.at[0])
        x_batch = lax.broadcasted_iota(jnp.int32, (rows, d), 0) // _HQ
        q_head = lax.broadcasted_iota(jnp.int32, (rows, _DH), 0) % _HQ
        for br in range(2):
            x = x_buf[br].astype(f32)
            x_rows = jnp.broadcast_to(x[0:1, :], (rows, d))
            for b in range(1, nb):
                x_rows = jnp.where(x_batch == b, x[b:b + 1, :], x_rows)

            def q_step(h, q, br=br, lhs=x_rows.astype(bf16)):
                w = wq_buf[br, :, pl.ds(pl.multiple_of(h * _DH, _DH), _DH)]
                return jnp.where(q_head == h, jnp.dot(lhs, w, preferred_element_type=f32), q)

            q = lax.fori_loop(0, _HQ, q_step, jnp.zeros((rows, _DH), f32), unroll=4)
            for b in range(nb):
                q_buf[br * nb + b] = q[b * _HQ:(b + 1) * _HQ].astype(bf16)
            start_a(_AHEAD - 2 + br)

        def attn_step(i, _):
            j = i + _AHEAD

            @pl.when(j < total_a)
            def _():
                start_a(j)

            @pl.when(jnp.logical_and(j >= total_a, j < total))
            def _():
                start_b(j)

            @pl.when(j >= total)
            def _():
                for t in range(_AHEAD):
                    @pl.when(j == total + t)
                    def _():
                        start_wo(t * _WO_ISSUED[0] // _AHEAD, (t + 1) * _WO_ISSUED[0] // _AHEAD)

            slot = i % nbuf
            g = jnp.where(i < total_a, i // steps_a, nb + (i - total_a) // steps_b)
            wait_all(kv_buf.at[slot], kv_sem.at[slot])

            qg = q_buf[g]
            kv_head = lax.broadcasted_iota(jnp.int32, (_HQ, _CHUNK), 0) // rep
            s = None
            for h in range(hkv):
                sh = lax.dot_general(qg, kv_buf[slot, 0, h], _NT, preferred_element_type=f32)
                s = sh if s is None else jnp.where(kv_head == h, sh, s)
            s = s * scale
            m_old = m_buf[g]
            m_new = jnp.maximum(m_old, jnp.max(s, axis=1, keepdims=True))
            alpha = jnp.exp(m_old - m_new)
            p = jnp.exp(s - m_new)
            m_buf[g] = m_new
            l_buf[g] = alpha * l_buf[g] + p
            pv = None
            for h in range(hkv):
                ph = jnp.where(kv_head == h, p, 0.0).astype(bf16)
                t = jnp.dot(ph, kv_buf[slot, 1, h], preferred_element_type=f32)
                pv = t if pv is None else pv + t
            acc_buf[g] = jnp.tile(alpha, (1, _DH // _CHUNK)) * acc_buf[g] + pv

        lax.fori_loop(0, total, attn_step, None)

        for g in range(2 * nb):
            acc_buf[g] = acc_buf[g] / jnp.sum(l_buf[g], axis=1, keepdims=True)

        def o_cols(br, c, n):
            w = min(n, _DH)
            lanes = slice(0, _DH) if n >= _DH else slice(c % _DH, c % _DH + n)
            row = lax.broadcasted_iota(jnp.int32, (8, w), 0)
            parts = []
            for t in range(n // w):
                part = jnp.zeros((8, w), f32)
                for b in range(nb):
                    head = acc_buf[br * nb + b, pl.ds(c // _DH + t, 1), lanes]
                    part = jnp.where(row == b, head, part)
                parts.append(part.astype(bf16))
            return jnp.concatenate(parts, axis=1)

        def project(r, o, c, n):
            return tuple(
                r[br] + lax.dot_general(o[br], wo_buf[pl.ds(wo_row0[br], d_pad), pl.ds(c, n)],
                                        _NT, preferred_element_type=f32)
                for br in range(2))

        per_block = _WO_BLOCK // _WO_STEP

        def o_step(k, r):
            for t in range(n_lead * per_block):
                @pl.when(k == t)
                def _():
                    start_wo(_WO_ISSUED[t], _WO_ISSUED[t + 1])

            c = pl.multiple_of(k * _WO_STEP, _WO_STEP)
            o = [o_cols(br, c, _WO_STEP) for br in range(2)]

            @pl.when(k % per_block == 0)
            def _():
                u = k // per_block
                cols = pl.ds(pl.multiple_of(u * _WO_BLOCK, _WO_BLOCK), _WO_BLOCK)
                wait_all(wo_buf.at[:, cols], wo_sem.at[u])

            return project(r, o, c, _WO_STEP)

        r = lax.fori_loop(0, n_lead * per_block, o_step, (jnp.zeros((8, d_pad), f32),) * 2)
        for u in range(n_lead, len(wo_widths)):
            c, n = wo_starts[u], wo_widths[u]
            o = [o_cols(br, c, n) for br in range(2)]
            wait_all(wo_buf.at[:, pl.ds(c, n)], wo_sem.at[u])
            r = project(r, o, c, n)

        lo = wo_row0[1]
        lane = lax.broadcasted_iota(jnp.int32, (8, d_pad - lo), 1)
        mid = jnp.where(lane < d - lo, r[0][:, lo:], r[1][:, :d_pad - lo])
        res = jnp.concatenate([r[0][:, :lo], mid, r[1][:, d_pad - lo:]], axis=1)
        o_ref[...] = res[:nb].astype(o_ref.dtype)

    out = pl.pallas_call(
        kernel_function,
        out_shape=jax.ShapeDtypeStruct((nb, 2 * d), bf16),
        in_specs=[pl.BlockSpec(memory_space=pltpu.HBM)] * 10,
        out_specs=pl.BlockSpec(memory_space=pltpu.VMEM),
        scratch_shapes=[
            pltpu.VMEM((nbuf, 2, hkv, _CHUNK, _DH), bf16),
            pltpu.VMEM((2, nb, d), bf16),
            pltpu.VMEM((2, d, _HQ * _DH), bf16),
            pltpu.VMEM((2 * d, _HQ * _DH), bf16),
            pltpu.VMEM((2 * nb, _HQ, _DH), bf16),
            pltpu.VMEM((2 * nb, _HQ, _CHUNK), f32),
            pltpu.VMEM((2 * nb, _HQ, _CHUNK), f32),
            pltpu.VMEM((2 * nb, _HQ, _DH), f32),
            pltpu.SemaphoreType.DMA((nbuf,)),
            pltpu.SemaphoreType.DMA((len(wo_widths),)),
            pltpu.SemaphoreType.DMA((1,)),
            pltpu.SemaphoreType.DMA((1,)),
        ],
        compiler_params=pltpu.CompilerParams(
            vmem_limit_bytes=32 * 1024 * 1024,
            disable_semaphore_checks=True,
        ),
    )(
        A_x.reshape(nb, d), A_k_cache, A_v_cache, A_wq, A_wo.T,
        B_x.reshape(nb, d), B_k_cache, B_v_cache, B_wq, B_wo.T,
    )
    return out.reshape(nb, 1, 2 * d)
```
